```python
import jax
import jax.numpy as jnp

def _softmax(x, axis=-1):
    return jax.nn.softmax(x, axis=axis)
def _gelu(x):
    return jax.nn.gelu(x, approximate=True)
def _silu(x):
    return jax.nn.silu(x)
def _sigmoid(x):
    return jax.nn.sigmoid(x)
def _layernorm(x, axis=-1, eps=1e-5):
    m = jnp.mean(x, axis=axis, keepdims=True)
    v = jnp.var(x, axis=axis, keepdims=True)
    return (x - m) / jnp.sqrt(v + eps)
def _scatter_add(tgt, idx, src, axis=0):
    return tgt.at[idx].add(src)
def _segment_sum(src, seg, n):
    return jax.ops.segment_sum(src, seg, n)
class _Rng:
    def __init__(self, key):
        self._k = key
    def _next(self):
        self._k, sub = jax.random.split(self._k)
        return sub
    def normal(self, shape):
        return jax.random.normal(self._next(), shape, dtype=jnp.bfloat16)
    def randint(self, lo, hi, shape):
        return jax.random.randint(self._next(), shape, lo, hi, dtype=jnp.int32)
    def uniform(self, shape, lo=0.0, hi=1.0):
        return jax.random.uniform(self._next(), shape, jnp.bfloat16, lo, hi)
    def permutation(self, n):
        return jax.random.permutation(self._next(), n)


kernel_name = 'sequential_preLN__mha_block_cached__moe_arch_mod__decode'

def setup_inputs():
    _rng = _Rng(jax.random.key(int.from_bytes(__import__("os").urandom(4), "little")))
    _w = (lambda a: (lambda t: t.astype(jnp.bfloat16) if jnp.issubdtype(t.dtype, jnp.floating) else t)(jnp.asarray(a)))
    def _A_setup():
        B, Sq, D = 4, 1, 640
        H, Sk, Dh = 32, 8192, 192
        return {
            "x": _w((lambda *s: _rng.normal(s) * 0.05)(B, Sq, D)),
            "k_cache": _w((lambda *s: _rng.normal(s) * 0.05)(B, H, Sk, Dh)),
            "v_cache": _w((lambda *s: _rng.normal(s) * 0.05)(B, H, Sk, Dh)),
            "wq": _w((lambda *s: _rng.normal(s) * 0.05)(D, H * Dh) * (D ** -0.5)),
            "wo": _w((lambda *s: _rng.normal(s) * 0.05)(H * Dh, D) * ((H * Dh) ** -0.5)),
        }
    _A_in = _A_setup()

    def _B_setup():
        B, S, D, F, C = 4, 1, 640, 1536, 1
        return {
            "x": _w((lambda *s: _rng.normal(s) * 0.05)(B, S, D)),
            "w_r": _w((lambda *s: _rng.normal(s) * 0.05)(D)),
            "w_gate": _w((lambda *s: _rng.normal(s) * 0.05)(D, F)),
            "w_up": _w((lambda *s: _rng.normal(s) * 0.05)(D, F)),
            "w_down": _w((lambda *s: _rng.normal(s) * 0.05)(F, D)),
        }
    _B_in = _B_setup()

    return {
        "A_x": _A_in["x"],
        "A_k_cache": _A_in["k_cache"],
        "A_v_cache": _A_in["v_cache"],
        "A_wq": _A_in["wq"],
        "A_wo": _A_in["wo"],
        "B_x": _B_in["x"],
        "B_w_r": _B_in["w_r"],
        "B_w_gate": _B_in["w_gate"],
        "B_w_up": _B_in["w_up"],
        "B_w_down": _B_in["w_down"],
    }

def reference(A_x, A_k_cache, A_v_cache, A_wq, A_wo, B_x, B_w_r, B_w_gate, B_w_up, B_w_down):
    def _A_ref(x, k_cache, v_cache, wq, wo):
        B, Sq, D = x.shape
        H, Dh = 32, 192
        q = (lambda x, *d: x.transpose(*d))((x @ wq).reshape(B, Sq, H, Dh), 0, 2, 1, 3)
        scores = jnp.einsum("bhqd,bhkd->bhqk", q, k_cache) * (Dh ** -0.5)
        p = _softmax(scores, axis=-1)
        o = jnp.einsum("bhqk,bhkd->bhqd", p, v_cache)
        return (lambda x, *d: x.transpose(*d))(o, 0, 2, 1, 3).reshape(B, Sq, H * Dh) @ wo

    def _B_ref(x, w_r, w_gate, w_up, w_down):
        B, S, D = x.shape
        C = 1
        r = x @ w_r
        idx = jnp.argsort(-r, axis=-1)[:, :C]
        idx_e = jnp.repeat(idx.reshape(B, C, 1), D, axis=2)
        x_sel = jnp.take_along_axis(x, idx_e, axis=1)
        g = _silu(x_sel @ w_gate)
        u = x_sel @ w_up
        y = (g * u) @ w_down
        r_sel = _sigmoid(jnp.take_along_axis(r, idx, axis=1))
        y = y * r_sel.reshape(B, C, 1)
        b_off = (jnp.arange(B) * S).reshape(B, 1)
        flat_idx = (idx + b_off).reshape(B * C)
        zero = (x * 0.0).reshape(B * S, D)
        upd = _scatter_add(zero, flat_idx, y.reshape(B * C, D), axis=0)
        return x + upd.reshape(B, S, D)

    x = A_x
    h = x + _A_ref(_layernorm(x, axis=-1), A_k_cache, A_v_cache, A_wq, A_wo)
    h2 = h + _B_ref(_layernorm(h, axis=-1), B_w_r, B_w_gate, B_w_up, B_w_down)
    return h2
```

```python
import functools

import jax
import jax.numpy as jnp
import jax.experimental.pallas as pl
import jax.experimental.pallas.tpu as pltpu

_EPS = 1e-5
_HP = 4
_CW = 1024
_RUNS = 2
_ORDER = (0, 2, 4, 1, 3, 5)
_AHEAD = (0, 9, 0, 9, 0, 9)
_NB = 3
_FW = 256
_TAIL = (1, 1)


def _layernorm(x):
    m = jnp.mean(x, axis=-1, keepdims=True)
    d = x - m
    v = jnp.mean(d * d, axis=-1, keepdims=True)
    return d / jnp.sqrt(v + _EPS)


def _dot(a, b):
    return jnp.dot(a, b, preferred_element_type=jnp.float32)


def _dot_nt(a, b):
    return jax.lax.dot_general(
        a, b, (((1,), (1,)), ((), ())), preferred_element_type=jnp.float32
    )


def _wait_all(buf, sem):
    pltpu.make_async_copy(buf, buf, sem).wait()


def _ds(start, size, align):
    return pl.ds(pl.multiple_of(start, align), size)


def _loop(n, body):
    jax.lax.fori_loop(0, n, lambda i, carry: body(i), None)


def _body(
    x_hbm, kt_hbm, vt_hbm, wq_hbm, wo_hbm, wr_hbm, wg_hbm, wu_hbm, wd_hbm,
    out_ref,
    ring, wqbuf, wobuf, wgbuf, wubuf, wdbuf, xbuf, wrbuf,
    q_scr, o_scr, acc_scr, s_scr, attn_scr,
    csem, wqsem, wosem, msem, gsem, dsem,
    *, B, H, Dh, Sk, D, F,
):
    P = _HP * Dh
    J = Sk // _CW
    HG = H // _HP
    n_steps = B * HG
    RT = ring.shape[3]
    NF = F // _FW
    scale = Dh ** -0.5

    def issue_cache(src, t, slot, j):
        def one_round(i):
            for k, (m, ahead) in enumerate(zip(_ORDER, _AHEAD)):
                pos = (j * RT + i + ahead) & (RT * J - 1)
                cols = _ds((pos & (J - 1)) * _CW, _CW, _CW)
                tile = pos >> (J.bit_length() - 1)
                pltpu.make_async_copy(
                    src.at[t, m, :, tile, :, cols],
                    ring.at[slot, m, :, tile, :, cols],
                    csem.at[slot],
                ).start(priority=k % 2)

        _loop(RT, one_round)

    def issue_wq(i):
        cols = _ds((i % 3) * 2048, 2048, 2048)
        for m in range(16):
            rows = _ds(((7 * m) % 16) * 40 + (i // 3) * 8, 8, 8)
            pltpu.make_async_copy(
                wq_hbm.at[rows, cols], wqbuf.at[rows, cols], wqsem.at[0]
            ).start(priority=m % 2)

    def issue_wo(i):
        for m in range(16):
            rows = _ds(((7 * m) % 16) * 384 + i * 32, 32, 32)
            pltpu.make_async_copy(
                wo_hbm.at[rows, :], wobuf.at[rows, :], wosem.at[0]
            ).start(priority=m % 2)

    def issue_gate_up(i):
        for m in range(8):
            rows = _ds(((3 * m) % 8) * 80 + i * 8, 8, 8)
            for k, (src, dst) in enumerate(((wg_hbm, wgbuf), (wu_hbm, wubuf))):
                pltpu.make_async_copy(
                    src.at[rows, :], dst.at[rows, :], gsem.at[0]
                ).start(priority=k)

    def issue_down(f):
        for i, r in enumerate(range(0, _FW, 32)):
            pltpu.make_async_copy(
                wd_hbm.at[_ds(f * _FW + r, 32, 32), :],
                wdbuf.at[f, pl.ds(r, 32), :],
                dsem.at[f],
            ).start(priority=i % 2)

    def issue_tail(first, count):
        def piece(i):
            i = first + i
            pl.when(i < 12)(lambda: issue_wo(i))
            pl.when(jnp.logical_and(i >= 12, i < 22))(lambda: issue_gate_up(i - 12))
            pl.when(jnp.logical_and(i >= 22, i < 22 + NF))(lambda: issue_down(i - 22))

        _loop(count, piece)

    x_cp = pltpu.make_async_copy(x_hbm, xbuf, msem.at[0])
    wr_cp = pltpu.make_async_copy(wr_hbm, wrbuf, msem.at[1])
    x_cp.start()
    wr_cp.start(priority=1)
    _loop(15, issue_wq)
    _loop(J, lambda j: issue_cache(kt_hbm, 0, 0, j))

    x_cp.wait()
    x4 = xbuf[...].astype(jnp.float32)
    x = jnp.concatenate([x4, x4], axis=0)
    xn = _layernorm(x).astype(jnp.bfloat16)
    o_scr[...] = jnp.zeros_like(o_scr)
    _wait_all(wqbuf, wqsem.at[0])

    def project_q(j):
        issue_cache(vt_hbm, 0, 1, j)
        pl.when(j < HG)(lambda: project(j))

    def project(hg):
        q_scr[hg] = _dot(xn, wqbuf[:, _ds(hg * P, P, P)])

    _loop(J, project_q)

    row = jax.lax.broadcasted_iota(jnp.int32, (8, P), 0)
    col = jax.lax.broadcasted_iota(jnp.int32, (8, P), 1)
    own = jnp.logical_and(col >= row * Dh, col < (row + 1) * Dh)

    def slab(slot, j):
        return ring[slot, :, :, :, :, _ds(j * _CW, _CW, _CW)].reshape(P, _CW)

    def step(t):
        b = t // HG
        hg = t % HG
        k_slot = (2 * t) % _NB
        v_slot = (2 * t + 1) % _NB
        more = t + 1 < n_steps
        last = jnp.logical_not(more)

        q = jnp.broadcast_to(q_scr[hg, pl.ds(b, 1), :], (8, P))
        q = jnp.where(own, q, 0.0).astype(jnp.bfloat16)
        _wait_all(ring.at[k_slot], csem.at[k_slot])

        def scores(j):
            pl.when(more)(lambda: issue_cache(kt_hbm, t + 1, (2 * t + 2) % _NB, j))
            pl.when(last)(lambda: issue_tail(j * _TAIL[0], _TAIL[0]))
            s_scr[j] = _dot(q, slab(k_slot, j)) * scale

        _loop(J, scores)

        s = s_scr[...]
        e = jnp.exp(s - jnp.max(jnp.max(s, axis=0), axis=-1, keepdims=True))
        s_scr[...] = e
        total = jnp.sum(jnp.sum(e, axis=0), axis=-1, keepdims=True)
        acc_scr[...] = jnp.zeros_like(acc_scr)
        _wait_all(ring.at[v_slot], csem.at[v_slot])

        def values(j):
            pl.when(more)(lambda: issue_cache(vt_hbm, t + 1, (2 * t + 3) % _NB, j))
            pl.when(last)(lambda: issue_tail(J * _TAIL[0] + j * _TAIL[1], _TAIL[1]))
            acc_scr[...] += _dot_nt(s_scr[j].astype(jnp.bfloat16), slab(v_slot, j))

        _loop(J, values)

        o = jnp.where(own, acc_scr[...] / total, 0.0)
        o_scr[hg, pl.ds(b, 1), :] = jnp.sum(o, axis=0, keepdims=True)

    _loop(n_steps, step)

    issued = J * sum(_TAIL)
    per_part = -(-max(22 + NF - issued, 0) // HG)
    attn_scr[...] = x
    _wait_all(wobuf, wosem.at[0])

    def project_out(hg):
        if per_part:
            issue_tail(issued + hg * per_part, per_part)
        attn_scr[...] += _dot(o_scr[hg].astype(jnp.bfloat16), wobuf[_ds(hg * P, P, P), :])

    _loop(HG, project_out)

    h = attn_scr[...]
    hn = _layernorm(h)
    hb = hn.astype(jnp.bfloat16)
    wr_cp.wait()
    r = jnp.sum(hn * wrbuf[...].astype(jnp.float32).reshape(1, D), axis=-1, keepdims=True)
    _wait_all(wgbuf, gsem.at[0])
    _wait_all(wubuf, gsem.at[0])
    gate = _dot(hb, wgbuf[...])
    up = _dot(hb, wubuf[...])
    act = (gate * jax.nn.sigmoid(gate) * up).astype(jnp.bfloat16)
    weight = jax.nn.sigmoid(r)
    y = jnp.zeros((2 * B, D), jnp.float32)
    for f in range(NF):
        _wait_all(wdbuf.at[f], dsem.at[f])
        y = y + _dot(act[:, f * _FW:(f + 1) * _FW], wdbuf[f])
    out = h + (hn + (hn * 0.0 + y * weight))
    out_ref[...] = out[:B].astype(out_ref.dtype)


@jax.jit
def pallas_sequential_preLN__mha_block_cached__moe_arch_mod__decode_kernel(
    A_x: jax.Array,
    A_k_cache: jax.Array,
    A_v_cache: jax.Array,
    A_wq: jax.Array,
    A_wo: jax.Array,
    B_x: jax.Array,
    B_w_r: jax.Array,
    B_w_gate: jax.Array,
    B_w_up: jax.Array,
    B_w_down: jax.Array,
):
    del B_x
    B, Sq, D = A_x.shape
    _, H, Sk, Dh = A_k_cache.shape
    F = B_w_gate.shape[1]
    assert (B, Sq, D, H, Sk, Dh, F) == (4, 1, 640, 32, 8192, 192, 1536)
    P = _HP * Dh
    chunk = (len(_ORDER), _RUNS, P // (8 * len(_ORDER) * _RUNS), 8, Sk)
    dt = A_k_cache.dtype
    f32 = jnp.float32

    kt = jnp.swapaxes(A_k_cache, 2, 3).reshape(B * H // _HP, *chunk)
    vt = jnp.swapaxes(A_v_cache, 2, 3).reshape(B * H // _HP, *chunk)

    out = pl.pallas_call(
        functools.partial(_body, B=B, H=H, Dh=Dh, Sk=Sk, D=D, F=F),
        in_specs=[pl.BlockSpec(memory_space=pl.ANY)] * 9,
        out_specs=pl.BlockSpec(memory_space=pltpu.VMEM),
        out_shape=jax.ShapeDtypeStruct((B, D), A_x.dtype),
        scratch_shapes=[
            pltpu.VMEM((_NB, *chunk), dt),
            pltpu.VMEM((D, H * Dh), dt),
            pltpu.VMEM((H * Dh, D), dt),
            pltpu.VMEM((D, F), dt),
            pltpu.VMEM((D, F), dt),
            pltpu.VMEM((F // _FW, _FW, D), dt),
            pltpu.VMEM((B, D), dt),
            pltpu.VMEM((D,), dt),
            pltpu.VMEM((H // _HP, 8, P), f32),
            pltpu.VMEM((H // _HP, 8, P), f32),
            pltpu.VMEM((8, P), f32),
            pltpu.VMEM((Sk // _CW, 8, _CW), f32),
            pltpu.VMEM((2 * B, D), f32),
            pltpu.SemaphoreType.DMA((_NB,)),
            pltpu.SemaphoreType.DMA((1,)),
            pltpu.SemaphoreType.DMA((1,)),
            pltpu.SemaphoreType.DMA((2,)),
            pltpu.SemaphoreType.DMA((1,)),
            pltpu.SemaphoreType.DMA((F // _FW,)),
        ],
        compiler_params=pltpu.CompilerParams(vmem_limit_bytes=100 * 1024 * 1024),
    )(A_x.reshape(B, D), kt, vt, A_wq, A_wo, B_w_r, B_w_gate, B_w_up, B_w_down)
    return out.reshape(B, Sq, D)
```

```python
import functools

import jax
import jax.numpy as jnp
import jax.experimental.pallas as pl
import jax.experimental.pallas.tpu as pltpu

_EPS = 1e-5
_HP = 4
_CW = 1024
_RUNS = 2
_ORDER = (3, 1, 4, 2, 0, 5)
_AHEAD = (0, 9, 0, 9, 1, 9)
_NB = 3
_DR = 64
_DW = 256
_DOWN = (0, 768, 1280, 1536)


def _layernorm(x):
    m = jnp.mean(x, axis=-1, keepdims=True)
    d = x - m
    v = jnp.mean(d * d, axis=-1, keepdims=True)
    return d / jnp.sqrt(v + _EPS)


def _dot(a, b):
    return jnp.dot(a, b, preferred_element_type=jnp.float32)


def _dot_nt(a, b):
    return jax.lax.dot_general(
        a, b, (((1,), (1,)), ((), ())), preferred_element_type=jnp.float32
    )


def _wait_all(buf, sem):
    pltpu.make_async_copy(buf, buf, sem).wait()


def _ds(start, size, align):
    return pl.ds(pl.multiple_of(start, align), size)


def _loop(n, body):
    jax.lax.fori_loop(0, n, lambda i, carry: body(i), None)


def _body(
    x_hbm, kt_hbm, vt_hbm, wq_hbm, wo_hbm, wr_hbm, wg_hbm, wu_hbm, wd_hbm,
    out_ref,
    ring, wqbuf, wobuf, wgbuf, wubuf, wdbuf, xbuf, wrbuf,
    q_scr, o_scr, acc_scr, s_scr, attn_scr, lhs_scr,
    csem, dsem,
    *, B, H, Dh, Sk, D, F,
):
    P = _HP * Dh
    J = Sk // _CW
    HG = H // _HP
    n_steps = B * HG
    RT = ring.shape[3]
    scale = Dh ** -0.5

    def issue_cache(src, t, slot, j):
        def one_round(i):
            for k, (m, ahead) in enumerate(zip(_ORDER, _AHEAD)):
                pos = (j * RT + i + ahead) & (RT * J - 1)
                cols = _ds((pos & (J - 1)) * _CW, _CW, _CW)
                tile = pos >> (J.bit_length() - 1)
                pltpu.make_async_copy(
                    src.at[t, m, :, tile, :, cols],
                    ring.at[slot, m, :, tile, :, cols],
                    csem.at[slot],
                ).start(priority=k % 2)

        _loop(RT, one_round)

    last_k = (2 * n_steps - 2) % _NB
    last_v = (2 * n_steps - 1) % _NB
    head_sem = csem.at[2]
    wo_sem = csem.at[(2 * n_steps) % _NB]
    up_sem = csem.at[last_k]
    down_sems = (csem.at[last_v], wo_sem) + tuple(dsem.at[i] for i in range(len(_DOWN) - 3))

    def issue_wq(i):
        cols = _ds((i % 3) * 2048, 2048, 2048)
        for m in range(16):
            rows = _ds(((7 * m) % 16) * 40 + (i // 3) * 8, 8, 8)
            pltpu.make_async_copy(
                wq_hbm.at[rows, cols], wqbuf.at[rows, cols], head_sem
            ).start(priority=m % 2)

    def issue_wo(i):
        for m in range(16):
            rows = _ds(((7 * m) % 16) * 384 + i * 32, 32, 32)
            pltpu.make_async_copy(
                wo_hbm.at[rows, :], wobuf.at[rows, :], wo_sem
            ).start(priority=m % 2)

    def issue_gate_up(row, priorities):
        rows = _ds(row, 8, 8)
        for src, dst, priority in zip((wg_hbm, wu_hbm), (wgbuf, wubuf), priorities):
            pltpu.make_async_copy(src.at[rows, :], dst.at[rows, :], up_sem).start(priority=priority)

    early = D // 8 - F // _DR

    def issue_early(i):
        def one(m):
            issue_gate_up((m * 8 + i) * 8, (0, 1))

        _loop(early // 8, one)

    def issue_down(f):
        def one(i):
            i = _DOWN[f] // _DR + i
            rows = _ds(i * _DR, _DR, _DR)
            issue_gate_up((early + i) * 8, (0, 0))
            pltpu.make_async_copy(
                wd_hbm.at[rows, :], wdbuf.at[rows, :], down_sems[f]
            ).start(priority=1)

        _loop((_DOWN[f + 1] - _DOWN[f]) // _DR, one)

    x_cp = pltpu.make_async_copy(x_hbm, xbuf, head_sem)
    wr_cp = pltpu.make_async_copy(wr_hbm, wrbuf, head_sem)
    _loop(15, issue_wq)
    x_cp.start()
    wr_cp.start()
    _loop(J, lambda j: issue_cache(kt_hbm, 0, 0, j))

    x_cp.wait()
    wr_cp.wait()
    _wait_all(wqbuf, head_sem)
    x4 = xbuf[...].astype(jnp.float32)
    x = jnp.concatenate([x4, x4], axis=0)
    xn = _layernorm(x).astype(jnp.bfloat16)
    o_scr[...] = jnp.zeros_like(o_scr)

    def project_q(j):
        issue_cache(vt_hbm, 0, 1, j)
        pl.when(j < HG)(lambda: project(j))

    def project(hg):
        q_scr[hg] = _dot(xn, wqbuf[:, _ds(hg * P, P, P)])

    _loop(J, project_q)

    row = jax.lax.broadcasted_iota(jnp.int32, (8, P), 0)
    col = jax.lax.broadcasted_iota(jnp.int32, (8, P), 1)
    own = jnp.logical_and(col >= row * Dh, col < (row + 1) * Dh)

    def slab(slot, j):
        return ring[slot, :, :, :, :, _ds(j * _CW, _CW, _CW)].reshape(P, _CW)

    def step(t):
        b = t // HG
        hg = t % HG
        k_slot = (2 * t) % _NB
        v_slot = (2 * t + 1) % _NB
        more = t + 1 < n_steps
        last = jnp.logical_not(more)

        q = jnp.broadcast_to(q_scr[hg, pl.ds(b, 1), :], (8, P))
        q = jnp.where(own, q, 0.0).astype(jnp.bfloat16)
        _wait_all(ring.at[k_slot], csem.at[k_slot])

        def scores(j):
            pl.when(more)(lambda: issue_cache(kt_hbm, t + 1, (2 * t + 2) % _NB, j))
            pl.when(last)(lambda: issue_wo(j))
            s_scr[j] = _dot(q, slab(k_slot, j)) * scale

        _loop(J, scores)

        s = s_scr[...]
        e = jnp.exp(s - jnp.max(jnp.max(s, axis=0), axis=-1, keepdims=True))
        s_scr[...] = e
        total = jnp.sum(jnp.sum(e, axis=0), axis=-1, keepdims=True)
        acc_scr[...] = jnp.zeros_like(acc_scr)
        _wait_all(ring.at[v_slot], csem.at[v_slot])

        def values(j):
            pl.when(more)(lambda: issue_cache(vt_hbm, t + 1, (2 * t + 3) % _NB, j))

            @pl.when(last)
            def _():
                pl.when(j < 4)(lambda: issue_wo(J + j))
                pl.when(j >= 4)(lambda: issue_early(j - 4))

            acc_scr[...] += _dot_nt(s_scr[j].astype(jnp.bfloat16), slab(v_slot, j))

        _loop(J, values)

        o = jnp.where(own, acc_scr[...] / total, 0.0)
        o_scr[hg, pl.ds(b, 1), :] = jnp.sum(o, axis=0, keepdims=True)

    _loop(n_steps, step)

    attn_scr[...] = x
    _wait_all(wobuf, wo_sem)

    def project_out(i):
        pl.when(i < 4)(lambda: issue_early(i + 4))
        pl.when(i == 4)(lambda: issue_down(0))
        pl.when(i == 6)(lambda: issue_down(1))
        attn_scr[...] += _dot(o_scr[i].astype(jnp.bfloat16), wobuf[_ds(i * P, P, P), :])

    _loop(HG, project_out)
    for f in range(2, len(_DOWN) - 1):
        issue_down(f)

    h = attn_scr[...]
    hn = _layernorm(h)
    r = jnp.sum(hn * wrbuf[...].astype(jnp.float32).reshape(1, D), axis=-1, keepdims=True)
    weight = jax.nn.sigmoid(r)
    for i in range(D // 128):
        lhs_scr[i] = hn[:, i * 128:(i + 1) * 128]

    def gate_up(i, carry):
        lhs = lhs_scr[i].astype(jnp.bfloat16)
        rows = _ds(i * 128, 128, 128)
        return carry[0] + _dot(lhs, wgbuf[rows, :]), carry[1] + _dot(lhs, wubuf[rows, :])

    _wait_all(wgbuf, up_sem)
    _wait_all(wubuf, up_sem)
    zero = jnp.zeros((8, F), jnp.float32)
    gate, up = jax.lax.fori_loop(0, D // 128, gate_up, (zero, zero))
    act = gate * jax.nn.sigmoid(gate) * up
    for i in range(F // 128):
        lhs_scr[i] = act[:, i * 128:(i + 1) * 128]

    def down(i, y):
        for lo, hi, sem in zip(_DOWN, _DOWN[1:], down_sems):
            pl.when(i == lo // _DW)(lambda: _wait_all(wdbuf.at[lo:hi], sem))
        for k in range(_DW // 128):
            c = i * (_DW // 128) + k
            y = y + _dot(lhs_scr[c].astype(jnp.bfloat16), wdbuf[_ds(c * 128, 128, 128), :])
        return y

    y = jax.lax.fori_loop(0, F // _DW, down, jnp.zeros((8, D), jnp.float32))
    out = h + (hn + (hn * 0.0 + y * weight))
    out_ref[...] = out[:B].astype(out_ref.dtype)


@jax.jit
def pallas_sequential_preLN__mha_block_cached__moe_arch_mod__decode_kernel(
    A_x: jax.Array,
    A_k_cache: jax.Array,
    A_v_cache: jax.Array,
    A_wq: jax.Array,
    A_wo: jax.Array,
    B_x: jax.Array,
    B_w_r: jax.Array,
    B_w_gate: jax.Array,
    B_w_up: jax.Array,
    B_w_down: jax.Array,
):
    del B_x
    B, Sq, D = A_x.shape
    _, H, Sk, Dh = A_k_cache.shape
    F = B_w_gate.shape[1]
    assert (B, Sq, D, H, Sk, Dh, F) == (4, 1, 640, 32, 8192, 192, 1536)
    P = _HP * Dh
    chunk = (len(_ORDER), _RUNS, P // (8 * len(_ORDER) * _RUNS), 8, Sk)
    dt = A_k_cache.dtype
    f32 = jnp.float32

    kt = jnp.swapaxes(A_k_cache, 2, 3).reshape(B * H // _HP, *chunk)
    vt = jnp.swapaxes(A_v_cache, 2, 3).reshape(B * H // _HP, *chunk)

    out = pl.pallas_call(
        functools.partial(_body, B=B, H=H, Dh=Dh, Sk=Sk, D=D, F=F),
        in_specs=[pl.BlockSpec(memory_space=pl.ANY)] * 9,
        out_specs=pl.BlockSpec(memory_space=pltpu.VMEM),
        out_shape=jax.ShapeDtypeStruct((B, D), A_x.dtype),
        scratch_shapes=[
            pltpu.VMEM((_NB, *chunk), dt),
            pltpu.VMEM((D, H * Dh), dt),
            pltpu.VMEM((H * Dh, D), dt),
            pltpu.VMEM((D, F), dt),
            pltpu.VMEM((D, F), dt),
            pltpu.VMEM((F, D), dt),
            pltpu.VMEM((B, D), dt),
            pltpu.VMEM((D,), dt),
            pltpu.VMEM((H // _HP, 8, P), f32),
            pltpu.VMEM((H // _HP, 8, P), f32),
            pltpu.VMEM((8, P), f32),
            pltpu.VMEM((Sk // _CW, 8, _CW), f32),
            pltpu.VMEM((8, D), f32),
            pltpu.VMEM((F // 128, 8, 128), f32),
            pltpu.SemaphoreType.DMA((_NB,)),
            pltpu.SemaphoreType.DMA((1,)),
        ],
        compiler_params=pltpu.CompilerParams(vmem_limit_bytes=100 * 1024 * 1024),
    )(A_x.reshape(B, D), kt, vt, A_wq, A_wo, B_w_r, B_w_gate, B_w_up, B_w_down)
    return out.reshape(B, Sq, D)
```

```python
import functools

import jax
import jax.numpy as jnp
import jax.experimental.pallas as pl
import jax.experimental.pallas.tpu as pltpu

_EPS = 1e-5
_HP = 4
_CW = 1024
_ORDER = (2, 1, 4, 3, 0, 5)
_AHEAD = (0, 9, 0, 9, 1, 9)
_NB = 3
_DR = 64
_DW = 256
_DOWN = (0, 768, 1280, 1536)


def _layernorm(x):
    m = jnp.mean(x, axis=-1, keepdims=True)
    d = x - m
    v = jnp.mean(d * d, axis=-1, keepdims=True)
    return d / jnp.sqrt(v + _EPS)


def _dot(a, b):
    return jnp.dot(a.astype(b.dtype), b, preferred_element_type=jnp.float32)


def _dot_nt(a, b):
    return jax.lax.dot_general(
        a.astype(b.dtype), b, (((1,), (1,)), ((), ())), preferred_element_type=jnp.float32
    )


def _wait_all(buf, sem):
    pltpu.make_async_copy(buf, buf, sem).wait()


def _ds(start, size, align):
    return pl.ds(pl.multiple_of(start, align), size)


def _loop(n, body):
    jax.lax.fori_loop(0, n, lambda i, carry: body(i), None)


def _body(
    x_hbm, kt_hbm, vt_hbm, wq_hbm, wo_hbm, wr_hbm, wg_hbm, wu_hbm, wd_hbm,
    out_ref,
    ring, wqbuf, wobuf, wgbuf, wubuf, wdbuf, xbuf, wrbuf,
    q_scr, o_scr, acc_scr, s_scr, h_scr, lhs_scr, sems,
    *, B, H, Dh, Sk, D, F,
):
    P = _HP * Dh
    J = Sk // _CW
    HG = H // _HP
    n_steps = B * HG
    RT = ring.shape[3]
    scale = Dh ** -0.5

    head_sem = sems.at[2]
    wo_sem = sems.at[(2 * n_steps) % _NB]
    up_sem = sems.at[(2 * n_steps - 2) % _NB]
    down_sems = (sems.at[(2 * n_steps - 1) % _NB], wo_sem, sems.at[_NB])

    def issue_cache(src, t, slot, j):
        def one_round(i):
            for k, (m, ahead) in enumerate(zip(_ORDER, _AHEAD)):
                pos = (j * RT + i + ahead) & (RT * J - 1)
                cols = _ds((pos & (J - 1)) * _CW, _CW, _CW)
                tile = pos >> (J.bit_length() - 1)
                pltpu.make_async_copy(
                    src.at[t, m, :, tile, :, cols],
                    ring.at[slot, m, :, tile, :, cols],
                    sems.at[slot],
                ).start(priority=k % 2)

        _loop(RT, one_round)

    def issue_wq(i):
        cols = _ds((i % 3) * 2048, 2048, 2048)
        for m in range(16):
            rows = _ds(((7 * m) % 16) * 40 + (i // 3) * 8, 8, 8)
            pltpu.make_async_copy(
                wq_hbm.at[rows, cols], wqbuf.at[rows, cols], head_sem
            ).start(priority=m % 2)

    def issue_wo(i):
        for m in range(16):
            rows = _ds(((7 * m) % 16) * 384 + i * 32, 32, 32)
            pltpu.make_async_copy(
                wo_hbm.at[rows, :], wobuf.at[rows, :], wo_sem
            ).start(priority=m % 2)

    def issue_gate_up(tile, priorities):
        rows = _ds(tile * 8, 8, 8)
        for src, dst, priority in zip((wg_hbm, wu_hbm), (wgbuf, wubuf), priorities):
            pltpu.make_async_copy(
                src.at[rows, :], dst.at[rows, :], up_sem
            ).start(priority=priority)

    early = D // 8 - F // _DR

    def issue_early(i):
        _loop(early // 8, lambda m: issue_gate_up(m * 8 + i, (0, 1)))

    def issue_down(f):
        def one(i):
            i = _DOWN[f] // _DR + i
            rows = _ds(i * _DR, _DR, _DR)
            issue_gate_up(early + i, (0, 0))
            pltpu.make_async_copy(
                wd_hbm.at[rows, :], wdbuf.at[rows, :], down_sems[f]
            ).start(priority=1)

        _loop((_DOWN[f + 1] - _DOWN[f]) // _DR, one)

    x_cp = pltpu.make_async_copy(x_hbm, xbuf, head_sem)
    wr_cp = pltpu.make_async_copy(wr_hbm, wrbuf, head_sem)
    _loop(15, issue_wq)
    x_cp.start()
    wr_cp.start()
    _loop(J, lambda j: issue_cache(kt_hbm, 0, 0, j))

    x_cp.wait()
    wr_cp.wait()
    _wait_all(wqbuf, head_sem)
    x4 = xbuf[...].astype(jnp.float32)
    x = jnp.concatenate([x4, x4], axis=0)
    xn = _layernorm(x)
    h_scr[...] = x
    o_scr[...] = jnp.zeros_like(o_scr)

    def project_q(hg):
        issue_cache(vt_hbm, 0, 1, hg)
        q_scr[hg] = _dot(xn, wqbuf[:, _ds(hg * P, P, P)])

    _loop(HG, project_q)

    row = jax.lax.broadcasted_iota(jnp.int32, (8, P), 0)
    col = jax.lax.broadcasted_iota(jnp.int32, (8, P), 1)
    own = jnp.logical_and(col >= row * Dh, col < (row + 1) * Dh)

    def slab(slot, j):
        return ring[slot, :, :, :, :, _ds(j * _CW, _CW, _CW)].reshape(P, _CW)

    def step(t):
        b = t // HG
        hg = t % HG
        k_slot = (2 * t) % _NB
        v_slot = (2 * t + 1) % _NB
        more = t + 1 < n_steps
        last = jnp.logical_not(more)

        q = jnp.broadcast_to(q_scr[hg, pl.ds(b, 1), :], (8, P))
        q = jnp.where(own, q, 0.0).astype(ring.dtype)
        _wait_all(ring.at[k_slot], sems.at[k_slot])

        def scores(j):
            pl.when(more)(lambda: issue_cache(kt_hbm, t + 1, (2 * t + 2) % _NB, j))
            pl.when(last)(lambda: issue_wo(j))
            s_scr[j] = _dot(q, slab(k_slot, j)) * scale

        _loop(J, scores)

        s = s_scr[...]
        e = jnp.exp(s - jnp.max(jnp.max(s, axis=0), axis=-1, keepdims=True))
        s_scr[...] = e
        total = jnp.sum(jnp.sum(e, axis=0), axis=-1, keepdims=True)
        acc_scr[...] = jnp.zeros_like(acc_scr)
        _wait_all(ring.at[v_slot], sems.at[v_slot])

        def values(j):
            pl.when(more)(lambda: issue_cache(vt_hbm, t + 1, (2 * t + 3) % _NB, j))

            @pl.when(last)
            def _():
                pl.when(j < 4)(lambda: issue_wo(J + j))
                pl.when(j >= 4)(lambda: issue_early(j - 4))

            acc_scr[...] += _dot_nt(s_scr[j], slab(v_slot, j))

        _loop(J, values)

        o = jnp.where(own, acc_scr[...] / total, 0.0)
        o_scr[hg, pl.ds(b, 1), :] = jnp.sum(o, axis=0, keepdims=True)

    _loop(n_steps, step)

    _wait_all(wobuf, wo_sem)

    def project_out(hg):
        pl.when(hg < 4)(lambda: issue_early(hg + 4))
        pl.when(hg == 4)(lambda: issue_down(0))
        pl.when(hg == 6)(lambda: issue_down(1))
        h_scr[...] += _dot(o_scr[hg], wobuf[_ds(hg * P, P, P), :])

    _loop(HG, project_out)
    issue_down(2)

    h = h_scr[...]
    hn = _layernorm(h)
    r = jnp.sum(hn * wrbuf[...].astype(jnp.float32).reshape(1, D), axis=-1, keepdims=True)
    weight = jax.nn.sigmoid(r)
    h_scr[...] = h + (hn + hn * 0.0)
    for i in range(D // 128):
        lhs_scr[i] = hn[:, i * 128:(i + 1) * 128]

    def gate_up(i, carry):
        rows = _ds(i * 128, 128, 128)
        return (
            carry[0] + _dot(lhs_scr[i], wgbuf[rows, :]),
            carry[1] + _dot(lhs_scr[i], wubuf[rows, :]),
        )

    _wait_all(wgbuf, up_sem)
    _wait_all(wubuf, up_sem)
    zero = jnp.zeros((8, F), jnp.float32)
    gate, up = jax.lax.fori_loop(0, D // 128, gate_up, (zero, zero))
    act = gate * jax.nn.sigmoid(gate) * up
    for i in range(_DOWN[2] // 128):
        lhs_scr[i] = act[:, i * 128:(i + 1) * 128]

    def wait_down(f):
        _wait_all(wdbuf.at[_DOWN[f]:_DOWN[f + 1]], down_sems[f])

    def down(i, y):
        pl.when(i == _DOWN[1] // _DW)(lambda: wait_down(1))
        for k in range(_DW // 128):
            c = i * (_DW // 128) + k
            y = y + _dot(lhs_scr[c], wdbuf[_ds(c * 128, 128, 128), :])
        return y

    wait_down(0)
    y = jax.lax.fori_loop(0, _DOWN[2] // _DW, down, jnp.zeros((8, D), jnp.float32))
    wait_down(2)
    y = y + _dot(act[:, _DOWN[2]:], wdbuf[_DOWN[2]:, :])
    out = h_scr[...] + y * weight
    out_ref[...] = out[:B].astype(out_ref.dtype)


@jax.jit
def pallas_sequential_preLN__mha_block_cached__moe_arch_mod__decode_kernel(
    A_x: jax.Array,
    A_k_cache: jax.Array,
    A_v_cache: jax.Array,
    A_wq: jax.Array,
    A_wo: jax.Array,
    B_x: jax.Array,
    B_w_r: jax.Array,
    B_w_gate: jax.Array,
    B_w_up: jax.Array,
    B_w_down: jax.Array,
):
    del B_x
    B, Sq, D = A_x.shape
    _, H, Sk, Dh = A_k_cache.shape
    F = B_w_gate.shape[1]
    assert (B, Sq, D, H, Sk, Dh, F) == (4, 1, 640, 32, 8192, 192, 1536)
    P = _HP * Dh
    chunk = (len(_ORDER), 2, P // (16 * len(_ORDER)), 8, Sk)
    dt = A_k_cache.dtype
    f32 = jnp.float32

    kt = jnp.swapaxes(A_k_cache, 2, 3).reshape(B * H // _HP, *chunk)
    vt = jnp.swapaxes(A_v_cache, 2, 3).reshape(B * H // _HP, *chunk)

    out = pl.pallas_call(
        functools.partial(_body, B=B, H=H, Dh=Dh, Sk=Sk, D=D, F=F),
        in_specs=[pl.BlockSpec(memory_space=pl.ANY)] * 9,
        out_specs=pl.BlockSpec(memory_space=pltpu.VMEM),
        out_shape=jax.ShapeDtypeStruct((B, D), A_x.dtype),
        scratch_shapes=[
            pltpu.VMEM((_NB, *chunk), dt),
            pltpu.VMEM((D, H * Dh), dt),
            pltpu.VMEM((H * Dh, D), dt),
            pltpu.VMEM((D, F), dt),
            pltpu.VMEM((D, F), dt),
            pltpu.VMEM((F, D), dt),
            pltpu.VMEM((B, D), dt),
            pltpu.VMEM((D,), dt),
            pltpu.VMEM((H // _HP, 8, P), f32),
            pltpu.VMEM((H // _HP, 8, P), f32),
            pltpu.VMEM((8, P), f32),
            pltpu.VMEM((Sk // _CW, 8, _CW), f32),
            pltpu.VMEM((8, D), f32),
            pltpu.VMEM((_DOWN[2] // 128, 8, 128), f32),
            pltpu.SemaphoreType.DMA((_NB + 1,)),
        ],
        compiler_params=pltpu.CompilerParams(
            vmem_limit_bytes=80 * 1024 * 1024, disable_bounds_checks=True
        ),
    )(A_x.reshape(B, D), kt, vt, A_wq, A_wo, B_w_r, B_w_gate, B_w_up, B_w_down)
    return out.reshape(B, Sq, D)
```

```python
import functools

import jax
import jax.numpy as jnp
import jax.experimental.pallas as pl
import jax.experimental.pallas.tpu as pltpu

_EPS = 1e-5
_HP = 4
_CW = 1024
_ORDER = (2, 1, 3, 4, 0, 5)
_AHEAD = (0, 9, 0, 9, 1, 9)
_NB = 3
_DR = 64
_DW = 256
_DOWN = (0, 768, 1280, 1536)


def _layernorm(x):
    m = jnp.mean(x, axis=-1, keepdims=True)
    d = x - m
    v = jnp.mean(d * d, axis=-1, keepdims=True)
    return d / jnp.sqrt(v + _EPS)


def _dot(a, b):
    return jnp.dot(a.astype(b.dtype), b, preferred_element_type=jnp.float32)


def _dot_nt(a, b):
    return jax.lax.dot_general(
        a.astype(b.dtype), b, (((1,), (1,)), ((), ())), preferred_element_type=jnp.float32
    )


def _wait_all(buf, sem):
    pltpu.make_async_copy(buf, buf, sem).wait()


def _ds(start, size, align):
    return pl.ds(pl.multiple_of(start, align), size)


def _loop(n, body):
    jax.lax.fori_loop(0, n, lambda i, carry: body(i), None)


def _body(
    x_hbm, kt_hbm, vt_hbm, wq_hbm, wo_hbm, wr_hbm, wg_hbm, wu_hbm, wd_hbm,
    out_ref,
    ring, wqbuf, wobuf, wgbuf, wubuf, wdbuf, xbuf, wrbuf,
    q_scr, o_scr, acc_scr, s_scr, h_scr, lhs_scr, sems,
    *, B, H, Dh, Sk, D, F,
):
    P = _HP * Dh
    J = Sk // _CW
    HG = H // _HP
    n_steps = B * HG
    RT = ring.shape[3]
    scale = Dh ** -0.5

    head_sem = sems.at[2]
    wo_sem = sems.at[(2 * n_steps) % _NB]
    up_sem = sems.at[(2 * n_steps - 2) % _NB]
    down_sems = (sems.at[(2 * n_steps - 1) % _NB], wo_sem, sems.at[_NB])

    def issue_cache(src, t, slot, j):
        def one_round(i):
            for k, (m, ahead) in enumerate(zip(_ORDER, _AHEAD)):
                pos = (j * RT + i + ahead) & (RT * J - 1)
                cols = _ds((pos & (J - 1)) * _CW, _CW, _CW)
                tile = pos >> (J.bit_length() - 1)
                pltpu.make_async_copy(
                    src.at[t, m, :, tile, :, cols],
                    ring.at[slot, m, :, tile, :, cols],
                    sems.at[slot],
                ).start(priority=k % 2)

        _loop(RT, one_round)

    def issue_wq(i):
        for m in range(wqbuf.shape[0]):
            pos = (i + 7 * (m % 2)) % 30
            at = (m, slice(None), pos // 6, slice(None), _ds((pos % 6) * 1024, 1024, 1024))
            pltpu.make_async_copy(
                wq_hbm.at[at], wqbuf.at[at], head_sem
            ).start(priority=m % 2)

    def issue_wo(piece):
        def one_round(i):
            for m in range(wobuf.shape[0]):
                pos = (4 * piece + i + 13 * (m % 2)) % 48
                pltpu.make_async_copy(
                    wo_hbm.at[m, :, pos], wobuf.at[m, :, pos], wo_sem
                ).start(priority=m % 2)

        _loop(4, one_round)

    def issue_gate_up(tile, priorities):
        rows = _ds(tile * 8, 8, 8)
        for src, dst, priority in zip((wg_hbm, wu_hbm), (wgbuf, wubuf), priorities):
            pltpu.make_async_copy(
                src.at[rows, :], dst.at[rows, :], up_sem
            ).start(priority=priority)

    early = D // 8 - F // _DR

    def issue_early(i):
        _loop(early // 8, lambda m: issue_gate_up(m * 8 + i, (0, 1)))

    def issue_down(f):
        def one(i):
            i = _DOWN[f] // _DR + i
            rows = _ds(i * _DR, _DR, _DR)
            issue_gate_up(early + i, (0, 0))
            pltpu.make_async_copy(
                wd_hbm.at[rows, :], wdbuf.at[rows, :], down_sems[f]
            ).start(priority=1)

        _loop((_DOWN[f + 1] - _DOWN[f]) // _DR, one)

    x_cp = pltpu.make_async_copy(x_hbm, xbuf, head_sem)
    wr_cp = pltpu.make_async_copy(wr_hbm, wrbuf, head_sem)
    _loop(30, issue_wq)
    x_cp.start()
    wr_cp.start()
    _loop(J, lambda j: issue_cache(kt_hbm, 0, 0, j))

    x_cp.wait()
    wr_cp.wait()
    _wait_all(wqbuf, head_sem)
    x4 = xbuf[...].astype(jnp.float32)
    x = jnp.concatenate([x4, x4], axis=0)
    xn = _layernorm(x)
    h_scr[...] = x
    o_scr[...] = jnp.zeros_like(o_scr)

    def project_q(hg):
        issue_cache(vt_hbm, 0, 1, hg)
        q_scr[hg] = _dot(xn, wqbuf[:, :, :, :, _ds(hg * P, P, P)].reshape(D, P))

    _loop(HG, project_q)

    row = jax.lax.broadcasted_iota(jnp.int32, (8, P), 0)
    col = jax.lax.broadcasted_iota(jnp.int32, (8, P), 1)
    own = jnp.logical_and(col >= row * Dh, col < (row + 1) * Dh)

    def slab(slot, j):
        return ring[slot, :, :, :, :, _ds(j * _CW, _CW, _CW)].reshape(P, _CW)

    def step(t):
        b = t // HG
        hg = t % HG
        k_slot = (2 * t) % _NB
        v_slot = (2 * t + 1) % _NB
        more = t + 1 < n_steps
        last = jnp.logical_not(more)

        q = jnp.broadcast_to(q_scr[hg, pl.ds(b, 1), :], (8, P))
        q = jnp.where(own, q, 0.0).astype(ring.dtype)
        _wait_all(ring.at[k_slot], sems.at[k_slot])

        def scores(j):
            pl.when(more)(lambda: issue_cache(kt_hbm, t + 1, (2 * t + 2) % _NB, j))
            pl.when(last)(lambda: issue_wo(j))
            s_scr[j] = _dot(q, slab(k_slot, j)) * scale

        _loop(J, scores)

        s = s_scr[...]
        e = jnp.exp(s - jnp.max(jnp.max(s, axis=0), axis=-1, keepdims=True))
        s_scr[...] = e
        total = jnp.sum(jnp.sum(e, axis=0), axis=-1, keepdims=True)
        acc_scr[...] = jnp.zeros_like(acc_scr)
        _wait_all(ring.at[v_slot], sems.at[v_slot])

        def values(j):
            pl.when(more)(lambda: issue_cache(vt_hbm, t + 1, (2 * t + 3) % _NB, j))

            @pl.when(last)
            def _():
                pl.when(j < 4)(lambda: issue_wo(J + j))
                pl.when(j >= 4)(lambda: issue_early(j - 4))

            acc_scr[...] += _dot_nt(s_scr[j], slab(v_slot, j))

        _loop(J, values)

        o = jnp.where(own, acc_scr[...] / total, 0.0)
        o_scr[hg, pl.ds(b, 1), :] = jnp.sum(o, axis=0, keepdims=True)

    _loop(n_steps, step)

    _wait_all(wobuf, wo_sem)

    def project_out(hg):
        pl.when(hg < 4)(lambda: issue_early(hg + 4))
        pl.when(hg == 4)(lambda: issue_down(0))
        pl.when(hg == 6)(lambda: issue_down(1))
        h_scr[...] += _dot(o_scr[hg], wobuf[hg // 2, pl.ds((hg % 2) * 2, 2)].reshape(P, D))

    _loop(HG, project_out)
    issue_down(2)

    h = h_scr[...]
    hn = _layernorm(h)
    r = jnp.sum(hn * wrbuf[...].astype(jnp.float32).reshape(1, D), axis=-1, keepdims=True)
    weight = jax.nn.sigmoid(r)
    h_scr[...] = h + (hn + hn * 0.0)
    for i in range(D // 128):
        lhs_scr[i] = hn[:, i * 128:(i + 1) * 128]

    def gate_up(i, carry):
        rows = _ds(i * 128, 128, 128)
        return (
            carry[0] + _dot(lhs_scr[i], wgbuf[rows, :]),
            carry[1] + _dot(lhs_scr[i], wubuf[rows, :]),
        )

    _wait_all(wgbuf, up_sem)
    _wait_all(wubuf, up_sem)
    zero = jnp.zeros((8, F), jnp.float32)
    gate, up = jax.lax.fori_loop(0, D // 128, gate_up, (zero, zero))
    act = gate * jax.nn.sigmoid(gate) * up
    for i in range(_DOWN[2] // 128):
        lhs_scr[i] = act[:, i * 128:(i + 1) * 128]

    def wait_down(f):
        _wait_all(wdbuf.at[_DOWN[f]:_DOWN[f + 1]], down_sems[f])

    def down(i, y):
        pl.when(i == _DOWN[1] // _DW)(lambda: wait_down(1))
        for k in range(_DW // 128):
            c = i * (_DW // 128) + k
            y = y + _dot(lhs_scr[c], wdbuf[_ds(c * 128, 128, 128), :])
        return y

    wait_down(0)
    y = jax.lax.fori_loop(0, _DOWN[2] // _DW, down, jnp.zeros((8, D), jnp.float32))
    wait_down(2)
    y = y + _dot(act[:, _DOWN[2]:], wdbuf[_DOWN[2]:, :])
    out = h_scr[...] + y * weight
    out_ref[...] = out[:B].astype(out_ref.dtype)


@jax.jit
def pallas_sequential_preLN__mha_block_cached__moe_arch_mod__decode_kernel(
    A_x: jax.Array,
    A_k_cache: jax.Array,
    A_v_cache: jax.Array,
    A_wq: jax.Array,
    A_wo: jax.Array,
    B_x: jax.Array,
    B_w_r: jax.Array,
    B_w_gate: jax.Array,
    B_w_up: jax.Array,
    B_w_down: jax.Array,
):
    del B_x
    B, Sq, D = A_x.shape
    _, H, Sk, Dh = A_k_cache.shape
    F = B_w_gate.shape[1]
    assert (B, Sq, D, H, Sk, Dh, F) == (4, 1, 640, 32, 8192, 192, 1536)
    P = _HP * Dh
    chunk = (len(_ORDER), 2, P // (16 * len(_ORDER)), 8, Sk)
    dt = A_k_cache.dtype
    f32 = jnp.float32

    kt = jnp.swapaxes(A_k_cache, 2, 3).reshape(B * H // _HP, *chunk)
    vt = jnp.swapaxes(A_v_cache, 2, 3).reshape(B * H // _HP, *chunk)
    wq = A_wq.reshape(8, 2, 5, 8, H * Dh)
    wo = A_wo.reshape(4, 4, 48, 8, D)

    out = pl.pallas_call(
        functools.partial(_body, B=B, H=H, Dh=Dh, Sk=Sk, D=D, F=F),
        in_specs=[pl.BlockSpec(memory_space=pl.ANY)] * 9,
        out_specs=pl.BlockSpec(memory_space=pltpu.VMEM),
        out_shape=jax.ShapeDtypeStruct((B, D), A_x.dtype),
        scratch_shapes=[
            pltpu.VMEM((_NB, *chunk), dt),
            pltpu.VMEM(wq.shape, dt),
            pltpu.VMEM(wo.shape, dt),
            pltpu.VMEM((D, F), dt),
            pltpu.VMEM((D, F), dt),
            pltpu.VMEM((F, D), dt),
            pltpu.VMEM((B, D), dt),
            pltpu.VMEM((D,), dt),
            pltpu.VMEM((H // _HP, 8, P), f32),
            pltpu.VMEM((H // _HP, 8, P), f32),
            pltpu.VMEM((8, P), f32),
            pltpu.VMEM((Sk // _CW, 8, _CW), f32),
            pltpu.VMEM((8, D), f32),
            pltpu.VMEM((_DOWN[2] // 128, 8, 128), f32),
            pltpu.SemaphoreType.DMA((_NB + 1,)),
        ],
        compiler_params=pltpu.CompilerParams(
            vmem_limit_bytes=80 * 1024 * 1024, disable_bounds_checks=True
        ),
    )(A_x.reshape(B, D), kt, vt, wq, wo, B_w_r, B_w_gate, B_w_up, B_w_down)
    return out.reshape(B, Sq, D)
```

```python
import functools

import jax
import jax.numpy as jnp
import jax.experimental.pallas as pl
import jax.experimental.pallas.tpu as pltpu

_EPS = 1e-5
_HP = 4
_CW = 1024
_ORDER = (2, 1, 3, 4, 0, 5)
_AHEAD = (0, 9, 0, 9, 1, 9)
_NB = 3
_DR = 64
_DW = 256
_DOWN = (0, 768, 1280, 1536)


def _layernorm(x):
    m = jnp.mean(x, axis=-1, keepdims=True)
    d = x - m
    v = jnp.mean(d * d, axis=-1, keepdims=True)
    return d / jnp.sqrt(v + _EPS)


def _dot(a, b):
    return jnp.dot(a.astype(b.dtype), b, preferred_element_type=jnp.float32)


def _dot_nt(a, b):
    return jax.lax.dot_general(
        a.astype(b.dtype), b, (((1,), (1,)), ((), ())), preferred_element_type=jnp.float32
    )


def _wait_all(buf, sem):
    pltpu.make_async_copy(buf, buf, sem).wait()


def _ds(start, size, align):
    return pl.ds(pl.multiple_of(start, align), size)


def _loop(n, body):
    jax.lax.fori_loop(0, n, lambda i, carry: body(i), None)


def _body(
    x_hbm, kt_hbm, vt_hbm, wq_hbm, wo_hbm, wr_hbm, wg_hbm, wu_hbm, wd_hbm,
    out_ref,
    ring, wqbuf, wobuf, wgbuf, wubuf, wdbuf, xbuf, wrbuf,
    q_scr, o_scr, acc_scr, s_scr, h_scr, lhs_scr, sems,
    *, B, H, Dh, Sk, D, F,
):
    P = _HP * Dh
    J = Sk // _CW
    HG = H // _HP
    n_steps = B * HG
    RT = ring.shape[3]
    scale = Dh ** -0.5

    head_sem = sems.at[2]
    wo_sem = sems.at[(2 * n_steps) % _NB]
    up_sem = sems.at[(2 * n_steps - 2) % _NB]
    down_sems = (sems.at[(2 * n_steps - 1) % _NB], wo_sem, sems.at[_NB])

    def issue_cache(src, t, slot, j):
        def one_round(i):
            for k, (m, ahead) in enumerate(zip(_ORDER, _AHEAD)):
                pos = (j * RT + i + ahead) & (RT * J - 1)
                cols = _ds((pos & (J - 1)) * _CW, _CW, _CW)
                tile = pos >> (J.bit_length() - 1)
                pltpu.make_async_copy(
                    src.at[t, m, :, tile, :, cols],
                    ring.at[slot, m, :, tile, :, cols],
                    sems.at[slot],
                ).start(priority=k % 2)

        _loop(RT, one_round)

    def issue_wq(i, fill):
        for m in range(wqbuf.shape[0]):
            pos = (i + 7 * (m % 2)) % 30
            at = (m, slice(None), pos // 6, slice(None), _ds((pos % 6) * 1024, 1024, 1024))
            pltpu.make_async_copy(
                wq_hbm.at[at], wqbuf.at[at], head_sem
            ).start(priority=1 if fill else m % 2)

    def issue_wo(piece):
        def one_round(i):
            for m in range(wobuf.shape[0]):
                pos = (4 * piece + i + 13 * (m % 2)) % 48
                pltpu.make_async_copy(
                    wo_hbm.at[m, :, pos], wobuf.at[m, :, pos], wo_sem
                ).start(priority=m % 2)

        _loop(4, one_round)

    def issue_gate_up(tile, priorities):
        tiles = (tile, (tile + D // 16) % (D // 8))
        for src, dst, at, priority in zip((wg_hbm, wu_hbm), (wgbuf, wubuf), tiles, priorities):
            rows = _ds(at * 8, 8, 8)
            pltpu.make_async_copy(
                src.at[rows, :], dst.at[rows, :], up_sem
            ).start(priority=priority)

    early = D // 8 - F // _DR

    def issue_early(i):
        _loop(early // 8, lambda m: issue_gate_up(m * 8 + i, (0, 1)))

    def issue_down(f):
        def one(i):
            i = _DOWN[f] // _DR + i
            rows = _ds(i * _DR, _DR, _DR)
            issue_gate_up(early + i, (0, 0))
            pltpu.make_async_copy(
                wd_hbm.at[rows, :], wdbuf.at[rows, :], down_sems[f]
            ).start(priority=1)

        _loop((_DOWN[f + 1] - _DOWN[f]) // _DR, one)

    x_cp = pltpu.make_async_copy(x_hbm, xbuf, head_sem)
    wr_cp = pltpu.make_async_copy(wr_hbm, wrbuf, head_sem)
    _loop(4, lambda i: issue_wq(i, True))
    _loop(26, lambda i: issue_wq(i + 4, False))
    x_cp.start()
    wr_cp.start()
    _loop(J, lambda j: issue_cache(kt_hbm, 0, 0, j))

    x_cp.wait()
    wr_cp.wait()
    _wait_all(wqbuf, head_sem)
    x4 = xbuf[...].astype(jnp.float32)
    x = jnp.concatenate([x4, x4], axis=0)
    xn = _layernorm(x)
    h_scr[...] = x
    o_scr[...] = jnp.zeros_like(o_scr)

    def project_q(hg):
        issue_cache(vt_hbm, 0, 1, hg)
        q_scr[hg] = _dot(xn, wqbuf[:, :, :, :, _ds(hg * P, P, P)].reshape(D, P))

    _loop(HG, project_q)

    row = jax.lax.broadcasted_iota(jnp.int32, (8, P), 0)
    col = jax.lax.broadcasted_iota(jnp.int32, (8, P), 1)
    own = jnp.logical_and(col >= row * Dh, col < (row + 1) * Dh)

    def slab(slot, j):
        return ring[slot, :, :, :, :, _ds(j * _CW, _CW, _CW)].reshape(P, _CW)

    def step(t):
        b = t // HG
        hg = t % HG
        k_slot = (2 * t) % _NB
        v_slot = (2 * t + 1) % _NB
        more = t + 1 < n_steps
        last = jnp.logical_not(more)

        q = jnp.broadcast_to(q_scr[hg, pl.ds(b, 1), :], (8, P))
        q = jnp.where(own, q, 0.0).astype(ring.dtype)
        _wait_all(ring.at[k_slot], sems.at[k_slot])

        def scores(j):
            pl.when(more)(lambda: issue_cache(kt_hbm, t + 1, (2 * t + 2) % _NB, j))
            pl.when(last)(lambda: issue_wo(j))
            s_scr[j] = _dot(q, slab(k_slot, j)) * scale

        _loop(J, scores)

        s = s_scr[...]
        e = jnp.exp(s - jnp.max(jnp.max(s, axis=0), axis=-1, keepdims=True))
        s_scr[...] = e
        total = jnp.sum(jnp.sum(e, axis=0), axis=-1, keepdims=True)
        acc_scr[...] = jnp.zeros_like(acc_scr)
        _wait_all(ring.at[v_slot], sems.at[v_slot])

        def values(j):
            pl.when(more)(lambda: issue_cache(vt_hbm, t + 1, (2 * t + 3) % _NB, j))

            @pl.when(last)
            def _():
                pl.when(j < 4)(lambda: issue_wo(J + j))
                pl.when(j >= 4)(lambda: issue_early(j - 4))

            acc_scr[...] += _dot_nt(s_scr[j], slab(v_slot, j))

        _loop(J, values)

        o = jnp.where(own, acc_scr[...] / total, 0.0)
        o_scr[hg, pl.ds(b, 1), :] = jnp.sum(o, axis=0, keepdims=True)

    _loop(n_steps, step)

    _wait_all(wobuf, wo_sem)

    def project_out(hg):
        pl.when(hg < 4)(lambda: issue_early(hg + 4))
        pl.when(hg == 4)(lambda: issue_down(0))
        pl.when(hg == 6)(lambda: issue_down(1))
        h_scr[...] += _dot(o_scr[hg], wobuf[hg // 2, pl.ds((hg % 2) * 2, 2)].reshape(P, D))

    _loop(HG, project_out)
    issue_down(2)

    h = h_scr[...]
    hn = _layernorm(h)
    r = jnp.sum(hn * wrbuf[...].astype(jnp.float32).reshape(1, D), axis=-1, keepdims=True)
    weight = jax.nn.sigmoid(r)
    h_scr[...] = h + (hn + hn * 0.0)
    for i in range(D // 128):
        lhs_scr[i] = hn[:, i * 128:(i + 1) * 128]

    def gate_up(i, carry):
        rows = _ds(i * 128, 128, 128)
        return (
            carry[0] + _dot(lhs_scr[i], wgbuf[rows, :]),
            carry[1] + _dot(lhs_scr[i], wubuf[rows, :]),
        )

    _wait_all(wgbuf, up_sem)
    _wait_all(wubuf, up_sem)
    zero = jnp.zeros((8, F), jnp.float32)
    gate, up = jax.lax.fori_loop(0, D // 128, gate_up, (zero, zero))
    act = gate * jax.nn.sigmoid(gate) * up
    for i in range(_DOWN[2] // 128):
        lhs_scr[i] = act[:, i * 128:(i + 1) * 128]

    def wait_down(f):
        _wait_all(wdbuf.at[_DOWN[f]:_DOWN[f + 1]], down_sems[f])

    def down(i, y):
        pl.when(i == _DOWN[1] // _DW)(lambda: wait_down(1))
        for k in range(_DW // 128):
            c = i * (_DW // 128) + k
            y = y + _dot(lhs_scr[c], wdbuf[_ds(c * 128, 128, 128), :])
        return y

    wait_down(0)
    y = jax.lax.fori_loop(0, _DOWN[2] // _DW, down, jnp.zeros((8, D), jnp.float32))
    wait_down(2)
    y = y + _dot(act[:, _DOWN[2]:], wdbuf[_DOWN[2]:, :])
    out = h_scr[...] + y * weight
    out_ref[...] = out[:B].astype(out_ref.dtype)


@jax.jit
def pallas_sequential_preLN__mha_block_cached__moe_arch_mod__decode_kernel(
    A_x: jax.Array,
    A_k_cache: jax.Array,
    A_v_cache: jax.Array,
    A_wq: jax.Array,
    A_wo: jax.Array,
    B_x: jax.Array,
    B_w_r: jax.Array,
    B_w_gate: jax.Array,
    B_w_up: jax.Array,
    B_w_down: jax.Array,
):
    del B_x
    B, Sq, D = A_x.shape
    _, H, Sk, Dh = A_k_cache.shape
    F = B_w_gate.shape[1]
    assert (B, Sq, D, H, Sk, Dh, F) == (4, 1, 640, 32, 8192, 192, 1536)
    P = _HP * Dh
    chunk = (len(_ORDER), 2, P // (16 * len(_ORDER)), 8, Sk)
    dt = A_k_cache.dtype
    f32 = jnp.float32

    kt = jnp.swapaxes(A_k_cache, 2, 3).reshape(B * H // _HP, *chunk)
    vt = jnp.swapaxes(A_v_cache, 2, 3).reshape(B * H // _HP, *chunk)
    wq = A_wq.reshape(8, 2, 5, 8, H * Dh)
    wo = A_wo.reshape(4, 4, 48, 8, D)

    out = pl.pallas_call(
        functools.partial(_body, B=B, H=H, Dh=Dh, Sk=Sk, D=D, F=F),
        in_specs=[pl.BlockSpec(memory_space=pl.ANY)] * 9,
        out_specs=pl.BlockSpec(memory_space=pltpu.VMEM),
        out_shape=jax.ShapeDtypeStruct((B, D), A_x.dtype),
        scratch_shapes=[
            pltpu.VMEM((_NB, *chunk), dt),
            pltpu.VMEM(wq.shape, dt),
            pltpu.VMEM(wo.shape, dt),
            pltpu.VMEM((D, F), dt),
            pltpu.VMEM((D, F), dt),
            pltpu.VMEM((F, D), dt),
            pltpu.VMEM((B, D), dt),
            pltpu.VMEM((D,), dt),
            pltpu.VMEM((H // _HP, 8, P), f32),
            pltpu.VMEM((H // _HP, 8, P), f32),
            pltpu.VMEM((8, P), f32),
            pltpu.VMEM((Sk // _CW, 8, _CW), f32),
            pltpu.VMEM((8, D), f32),
            pltpu.VMEM((_DOWN[2] // 128, 8, 128), f32),
            pltpu.SemaphoreType.DMA((_NB + 1,)),
        ],
        compiler_params=pltpu.CompilerParams(
            vmem_limit_bytes=80 * 1024 * 1024, disable_bounds_checks=True
        ),
    )(A_x.reshape(B, D), kt, vt, wq, wo, B_w_r, B_w_gate, B_w_up, B_w_down)
    return out.reshape(B, Sq, D)
```
